```python
import jax
import jax.numpy as jnp

def _softmax(x, axis=-1):
    return jax.nn.softmax(x, axis=axis)
def _gelu(x):
    return jax.nn.gelu(x, approximate=True)
def _silu(x):
    return jax.nn.silu(x)
def _sigmoid(x):
    return jax.nn.sigmoid(x)
def _layernorm(x, axis=-1, eps=1e-5):
    m = jnp.mean(x, axis=axis, keepdims=True)
    v = jnp.var(x, axis=axis, keepdims=True)
    return (x - m) / jnp.sqrt(v + eps)
def _scatter_add(tgt, idx, src, axis=0):
    return tgt.at[idx].add(src)
def _segment_sum(src, seg, n):
    return jax.ops.segment_sum(src, seg, n)
class _Rng:
    def __init__(self, key):
        self._k = key
    def _next(self):
        self._k, sub = jax.random.split(self._k)
        return sub
    def normal(self, shape):
        return jax.random.normal(self._next(), shape, dtype=jnp.bfloat16)
    def randint(self, lo, hi, shape):
        return jax.random.randint(self._next(), shape, lo, hi, dtype=jnp.int32)
    def uniform(self, shape, lo=0.0, hi=1.0):
        return jax.random.uniform(self._next(), shape, jnp.bfloat16, lo, hi)
    def permutation(self, n):
        return jax.random.permutation(self._next(), n)


kernel_name = 'standalone__detection_seg_fpn_lateral__vision'

def setup_inputs():
    _rng = _Rng(jax.random.key(int.from_bytes(__import__("os").urandom(4), "little")))
    _w = (lambda a: (lambda t: t.astype(jnp.bfloat16) if jnp.issubdtype(t.dtype, jnp.floating) else t)(jnp.asarray(a)))
    H = W = (384 // 2) * 2
    C = 384
    k = 1
    return {
        "c_fine": _w((lambda *s: _rng.normal(s) * 0.05)(1, H, W, C)),
        "p_coarse": _w((lambda *s: _rng.normal(s) * 0.05)(1, H // 2, W // 2, C)),
        "w_lat": _w((lambda *s: _rng.normal(s) * 0.05)(C, C)),
        "w_out": _w((lambda *s: _rng.normal(s) * 0.05)(k, k, C, C)),
    }

def reference(c_fine, p_coarse, w_lat, w_out):
    B, H, W, C = c_fine.shape
    k = 1
    lat = jnp.einsum("bhwc,cd->bhwd", c_fine, w_lat)
    up = jnp.repeat(jnp.repeat(p_coarse, 2, axis=1), 2, axis=2)
    m = lat + up
    pad = k // 2
    mp = jnp.pad(m, ((0, 0), (pad, pad), (pad, pad), (0, 0)))
    o = None
    for di in range(k):
        for dj in range(k):
            t = jnp.einsum("bhwc,cd->bhwd", mp[:, di:di + H, dj:dj + W, :], w_out[di, dj])
            o = t if o is None else o + t
    return o
```

```python
import jax
import jax.numpy as jnp
import jax.experimental.pallas as pl
import jax.experimental.pallas.tpu as pltpu

_BH = 8


def _kernel(c_ref, p_ref, wl_ref, wo_ref, o_ref, wc_ref):
    @pl.when(pl.program_id(0) == 0)
    def _():
        wc_ref[...] = jnp.dot(
            wl_ref[...], wo_ref[...], preferred_element_type=jnp.float32
        ).astype(wc_ref.dtype)

    for hp in range(c_ref.shape[0] // 2):
        q = jnp.dot(p_ref[hp], wo_ref[...], preferred_element_type=jnp.float32)
        qe = pltpu.bitcast(
            pltpu.pack_elementwise([q, q], packed_dtype=jnp.bfloat16), jnp.bfloat16
        ).astype(jnp.float32)
        for h in (2 * hp, 2 * hp + 1):
            acc = jnp.dot(c_ref[h], wc_ref[...], preferred_element_type=jnp.float32)
            o_ref[h] = (acc + qe).astype(o_ref.dtype)


@jax.jit
def pallas_standalone__detection_seg_fpn_lateral__vision_kernel(
    c_fine: jax.Array,
    p_coarse: jax.Array,
    w_lat: jax.Array,
    w_out: jax.Array,
):
    B, H, W, C = c_fine.shape
    D = w_out.shape[-1]
    rows = B * H
    out = pl.pallas_call(
        _kernel,
        grid=(rows // _BH,),
        in_specs=[
            pl.BlockSpec((_BH, W, C), lambda i: (i, 0, 0)),
            pl.BlockSpec((_BH // 2, W // 2, C), lambda i: (i, 0, 0)),
            pl.BlockSpec((C, C), lambda i: (0, 0)),
            pl.BlockSpec((C, D), lambda i: (0, 0)),
        ],
        out_specs=pl.BlockSpec((_BH, W, D), lambda i: (i, 0, 0)),
        out_shape=jax.ShapeDtypeStruct((rows, W, D), c_fine.dtype),
        scratch_shapes=[pltpu.VMEM((C, D), c_fine.dtype)],
        compiler_params=pltpu.CompilerParams(
            dimension_semantics=("arbitrary",),
            vmem_limit_bytes=100 * 1024 * 1024,
        ),
    )(
        c_fine.reshape(rows, W, C),
        p_coarse.reshape(rows // 2, W // 2, C),
        w_lat,
        w_out.reshape(C, D),
    )
    return out.reshape(B, H, W, D)
```

```python
import functools

import jax
import jax.numpy as jnp
from jax import lax
import jax.experimental.pallas as pl
import jax.experimental.pallas.tpu as pltpu

_LANES = 128
_GROUP = 3
_PIECE = 48
_UNITS = 4
_READ_LEAD, _READ_RATE = 3, 2
_WRITE_LEAD, _WRITE_RATE = 8, 3


def _upsample_w(q, up_ref):
    tiles = up_ref.shape[0]
    for t in range(tiles):
        for parity in range(2):
            rows = pl.ds(parity, q.shape[0], stride=2)
            up_ref[t, rows, :] = q[:, t * _LANES:(t + 1) * _LANES]
    return jnp.concatenate([up_ref[t] for t in range(tiles)], axis=1)


def _kernel(
    c_hbm, p_hbm, wl_hbm, wo_hbm, o_hbm,
    lo_ref, hi_ref, p_ref, wl_ref, wo_ref, wc_ref, up0_ref, up1_ref,
    lo_sem, hi_sem, p_sem, w_sem, o_sem,
    *, switch,
):
    n, pair_rows, _ = lo_ref.shape
    ring = p_ref.shape[0]
    width = pair_rows // 2
    unit_rows = pair_rows // _UNITS

    def read_lo(s):
        sem = lo_sem.at[lax.rem(s, ring)]
        return pltpu.make_async_copy(c_hbm.at[0, s], lo_ref.at[s], sem)

    def read_hi(s):
        sem = hi_sem.at[lax.rem(s, ring)]
        return pltpu.make_async_copy(c_hbm.at[1, s], hi_ref.at[s + 1], sem)

    def read_p(s):
        slot = lax.rem(s, ring)
        return pltpu.make_async_copy(p_hbm.at[:, s], p_ref.at[slot], p_sem.at[slot])

    def start_reads(first, last):
        @pl.loop(first, last)
        def _(s):
            for read in (read_lo, read_hi, read_p):
                read(s).start()

    def wait_reads(s):
        for read in (read_lo, read_hi, read_p):
            read(s).wait()

    def start_writes(first, last):
        @pl.loop(first, last)
        def _(u):
            group = lax.div(u, _UNITS)
            pairs = pl.ds(group * _GROUP, _GROUP)
            base = (u - group * _UNITS) * unit_rows
            for offset in range(0, unit_rows, _PIECE):
                rows = pl.ds(pl.multiple_of(base + offset, _PIECE), _PIECE)
                for half, src in enumerate((hi_ref, lo_ref)):
                    pltpu.make_async_copy(
                        src.at[pairs, rows], o_hbm.at[half, pairs, rows], o_sem
                    ).start()

    def reads_started(s):
        limit = jnp.minimum(n, s - 1 + ring)
        return jnp.minimum(limit, _READ_LEAD + _READ_RATE * s)

    def writes_started(s):
        ready = lax.div(s, _GROUP) * _UNITS
        paced = jnp.minimum(ready, _WRITE_LEAD + _WRITE_RATE * (s - switch))
        return jnp.where(s < switch, 0, paced)

    def compute_pair(src_ref, src, coarse, up_ref, dst_ref, dst):
        up = _upsample_w(
            jnp.dot(coarse, wo_ref[...], preferred_element_type=jnp.float32), up_ref
        )
        for rows in (pl.ds(0, width), pl.ds(width, width)):
            acc = jnp.dot(
                src_ref[src, rows], wc_ref[...], preferred_element_type=jnp.float32
            )
            dst_ref[dst, rows] = (acc + up).astype(dst_ref.dtype)

    weights = (
        pltpu.make_async_copy(wo_hbm, wo_ref, w_sem.at[0]),
        pltpu.make_async_copy(wl_hbm, wl_ref, w_sem.at[1]),
    )
    for copy in weights:
        copy.start()
    start_reads(0, min(n, ring - 1, _READ_LEAD))
    for copy in weights:
        copy.wait()
    wc_ref[...] = jnp.dot(
        wl_ref[...], wo_ref[...], preferred_element_type=jnp.float32
    ).astype(wc_ref.dtype)

    @pl.loop(0, n)
    def _(s):
        @pl.when(s < switch)
        def _():
            start_reads(reads_started(s), reads_started(s + 1))
            wait_reads(s)

        @pl.when(s == switch)
        def _():
            pl.loop(switch, n - 1)(wait_reads)
            read_lo(n - 1).wait()
            read_hi(n - 1).wait()

        @pl.when(s >= switch)
        def _():
            start_writes(writes_started(s - 1), writes_started(s))

        @pl.when(s == switch)
        def _():
            read_p(n - 1).wait()

        slot = lax.rem(s, ring)
        compute_pair(lo_ref, s, p_ref[slot, 0], up0_ref, hi_ref, s)
        compute_pair(hi_ref, s + 1, p_ref[slot, 1], up1_ref, lo_ref, s)

    start_writes(writes_started(n - 1), n // _GROUP * _UNITS)
    pltpu.make_async_copy(o_hbm, o_hbm, o_sem).wait()


@jax.jit
def pallas_standalone__detection_seg_fpn_lateral__vision_kernel(
    c_fine: jax.Array,
    p_coarse: jax.Array,
    w_lat: jax.Array,
    w_out: jax.Array,
):
    B, H, W, C = c_fine.shape
    dtype = c_fine.dtype
    n = B * H // 4
    assert w_lat.shape == (C, C) and w_out.shape == (1, 1, C, C)
    assert H % 2 == 0 and (B * H) % (4 * _GROUP) == 0
    assert (2 * W) % (_UNITS * _PIECE) == 0 and C % _LANES == 0
    switch = pl.cdiv(7 * n, 12)
    ring = n + 1 - switch

    out = pl.pallas_call(
        functools.partial(_kernel, switch=switch),
        in_specs=[pl.BlockSpec(memory_space=pl.ANY)] * 4,
        out_specs=pl.BlockSpec(memory_space=pl.ANY),
        out_shape=jax.ShapeDtypeStruct((2, n, 2 * W, C), dtype),
        scratch_shapes=[
            pltpu.VMEM((n, 2 * W, C), dtype),
            pltpu.VMEM((n + 1, 2 * W, C), dtype),
            pltpu.VMEM((ring, 2, W // 2, C), dtype),
            pltpu.VMEM((C, C), dtype),
            pltpu.VMEM((C, C), dtype),
            pltpu.VMEM((C, C), dtype),
            pltpu.VMEM((C // _LANES, W, _LANES), jnp.float32),
            pltpu.VMEM((C // _LANES, W, _LANES), jnp.float32),
            pltpu.SemaphoreType.DMA((ring,)),
            pltpu.SemaphoreType.DMA((ring,)),
            pltpu.SemaphoreType.DMA((ring,)),
            pltpu.SemaphoreType.DMA((2,)),
            pltpu.SemaphoreType.DMA(()),
        ],
        compiler_params=pltpu.CompilerParams(
            vmem_limit_bytes=126 * 1024 * 1024,
            disable_semaphore_checks=True,
        ),
    )(
        c_fine.reshape(2, n, 2 * W, C),
        p_coarse.reshape(2, n, W // 2, C),
        w_lat,
        w_out.reshape(C, C),
    )
    return out.reshape(B, H, W, C)
```
